```python
import jax
import jax.numpy as jnp

def _softmax(x, axis=-1):
    return jax.nn.softmax(x, axis=axis)
def _gelu(x):
    return jax.nn.gelu(x, approximate=True)
def _silu(x):
    return jax.nn.silu(x)
def _sigmoid(x):
    return jax.nn.sigmoid(x)
def _layernorm(x, axis=-1, eps=1e-5):
    m = jnp.mean(x, axis=axis, keepdims=True)
    v = jnp.var(x, axis=axis, keepdims=True)
    return (x - m) / jnp.sqrt(v + eps)
def _scatter_add(tgt, idx, src, axis=0):
    return tgt.at[idx].add(src)
def _segment_sum(src, seg, n):
    return jax.ops.segment_sum(src, seg, n)
class _Rng:
    def __init__(self, key):
        self._k = key
    def _next(self):
        self._k, sub = jax.random.split(self._k)
        return sub
    def normal(self, shape):
        return jax.random.normal(self._next(), shape, dtype=jnp.bfloat16)
    def randint(self, lo, hi, shape):
        return jax.random.randint(self._next(), shape, lo, hi, dtype=jnp.int32)
    def uniform(self, shape, lo=0.0, hi=1.0):
        return jax.random.uniform(self._next(), shape, jnp.bfloat16, lo, hi)
    def permutation(self, n):
        return jax.random.permutation(self._next(), n)


kernel_name = 'gated_mix__sliding_local_dilated__ssm_conv_s4__prompt'

def setup_inputs():
    _rng = _Rng(jax.random.key(int.from_bytes(__import__("os").urandom(4), "little")))
    _w = (lambda a: (lambda t: t.astype(jnp.bfloat16) if jnp.issubdtype(t.dtype, jnp.floating) else t)(jnp.asarray(a)))
    def _A_setup():
        B, S, D = 1, 2048, 640
        return {
            "x": _w((lambda *s: _rng.normal(s) * 0.05)(B, S, D)),
            "wqkv": _w((lambda *s: _rng.normal(s) * 0.05)(D, 3 * D)),
            "wo": _w((lambda *s: _rng.normal(s) * 0.05)(D, D)),
        }
    _A_in = _A_setup()

    def _B_setup():
        B, L, D, N = 1, 2048, 640, 192
        A_re = -jnp.exp((lambda *s: _rng.normal(s) * 0.05)(D, N))
        A_im = jnp.pi * (lambda *s: _rng.normal(s) * 0.05)(D, N)
        B_re = (lambda *s: _rng.normal(s) * 0.05)(D, N)
        B_im = (lambda *s: _rng.normal(s) * 0.05)(D, N)
        C_re = (lambda *s: _rng.normal(s) * 0.05)(D, N)
        C_im = (lambda *s: _rng.normal(s) * 0.05)(D, N)
        log_dt = (lambda *s: _rng.normal(s) * 0.05)(D) * 0.5 - 4.0
        Dskip = (lambda *s: _rng.normal(s) * 0.05)(D)
        return {
            "u": _w((lambda *s: _rng.normal(s) * 0.05)(B, L, D)),
            "A_re": _w(A_re),
            "A_im": _w(A_im),
            "B_re": _w(B_re),
            "B_im": _w(B_im),
            "C_re": _w(C_re),
            "C_im": _w(C_im),
            "log_dt": _w(log_dt),
            "Dskip": _w(Dskip),
        }
    _B_in = _B_setup()

    return {
        "A_x": _A_in["x"],
        "A_wqkv": _A_in["wqkv"],
        "A_wo": _A_in["wo"],
        "B_u": _B_in["u"],
        "B_A_re": _B_in["A_re"],
        "B_A_im": _B_in["A_im"],
        "B_B_re": _B_in["B_re"],
        "B_B_im": _B_in["B_im"],
        "B_C_re": _B_in["C_re"],
        "B_C_im": _B_in["C_im"],
        "B_log_dt": _B_in["log_dt"],
        "B_Dskip": _B_in["Dskip"],
        "gate_w": _w((lambda *s: _rng.normal(s) * 0.05)(640)),
    }

def reference(A_x, A_wqkv, A_wo, B_u, B_A_re, B_A_im, B_B_re, B_B_im, B_C_re, B_C_im, B_log_dt, B_Dskip, gate_w):
    def _A_ref(x, wqkv, wo):
        B, S, D = x.shape
        H = 32; Dh = D // H
        W, dil = 8, 2
        qkv = (lambda x, *d: x.transpose(*d))((x @ wqkv).reshape(B, S, 3, H, Dh), 2, 0, 3, 1, 4)
        q, k, v = qkv[0], qkv[1], qkv[2]
        scale = Dh ** -0.5
        pos = jnp.arange(S)
        off = jnp.arange(W) * dil
        idx = pos[:, None] - off[None, :]
        mask = idx >= 0
        idx_c = jnp.where(mask, idx, 0).reshape(-1)
        kg = k[:, :, idx_c, :].reshape(B, H, S, W, Dh)
        vg = v[:, :, idx_c, :].reshape(B, H, S, W, Dh)
        logits = jnp.einsum("bhsd,bhswd->bhsw", q, kg) * scale
        logits = jnp.where(mask[None, None, :, :], logits, -1e9)
        attn = _softmax(logits, axis=-1)
        o = jnp.einsum("bhsw,bhswd->bhsd", attn, vg)
        return (lambda x, *d: x.transpose(*d))(o, 0, 2, 1, 3).reshape(B, S, D) @ wo

    def _B_ref(u, A_re, A_im, B_re, B_im, C_re, C_im, log_dt, Dskip):
        Bsz, L, D = u.shape
        dt = jnp.exp(log_dt)[:, None]
        A = A_re + 1j * A_im
        Bc = B_re + 1j * B_im
        Cc = C_re + 1j * C_im
        logdA = dt * A
        dB = dt * Bc
        l = (lambda x, dt: x.astype(dt))(jnp.arange(L), A_re.dtype)
        P = jnp.exp(logdA[:, :, None] * l[None, None, :])
        K = jnp.einsum("dn,dnl,dn->dl", Cc, P, dB).real
        L2 = 2 * L
        Kp = jnp.pad(K, ((0, 0), (0, L)))
        up = (lambda x, *d: x.transpose(*d))(u, 0, 2, 1)
        up = jnp.pad(up, ((0, 0), (0, 0), (0, L)))
        Kf = (lambda x, axes=(-2,-1): jnp.fft.rfft2(x.astype(jnp.float32), axes=axes))(Kp[:, None, :], axes=(-2, -1))
        Uf = (lambda x, axes=(-2,-1): jnp.fft.rfft2(x.astype(jnp.float32), axes=axes))(up[:, :, None, :], axes=(-2, -1))
        Yf = Uf * Kf[None, :, :, :]
        y = (lambda x, s, axes=(-2,-1): jnp.fft.irfft2(x, s=s, axes=axes).astype(jnp.bfloat16))(Yf, (1, L2), axes=(-2, -1))[:, :, 0, :L]
        y = (lambda x, *d: x.transpose(*d))(y, 0, 2, 1) + u * Dskip[None, None, :]
        return y

    x = A_x
    g = _sigmoid((x * gate_w).sum(-1, keepdims=True))
    a = _A_ref(x, A_wqkv, A_wo)
    b = _B_ref(x, B_A_re, B_A_im, B_B_re, B_B_im, B_C_re, B_C_im, B_log_dt, B_Dskip)
    return g * a + (1 - g) * b
```

```python
import functools

import jax
import jax.numpy as jnp
import numpy as np
import jax.experimental.pallas as pl
import jax.experimental.pallas.tpu as pltpu

S = 2048
D = 640
N = 192
H = 32
DH = D // H
WIN, DIL = 8, 2
HALO = 16
T = 128
NC = S // T
CT = D // 128
F32, BF16 = jnp.float32, jnp.bfloat16
RB = 256
MR = 128
MK = 128
AB = 256
AR = 16
CP = 2
HOPX, PF, PER_PRODUCT = 3, (0.8, 0.3), 250
H1, H2, H2_LAST = 34, 8, 4
H3, H3_W, H3_C, H3_LATE, H3_FIRST = 20, 3, 3, 56, 20
LOG2E = 1.4426950408889634
NT_DIMS = (((1,), (1,)), ((), ()))


def _round_bf16(v):
    u = np.asarray(v, np.float32).view(np.uint32)
    u = (u + 0x7FFF + ((u >> 16) & 1)) & 0xFFFF0000
    return u.view(np.float32)


def _pack_rows(m):
    bits = np.ascontiguousarray(_round_bf16(m)).view(np.uint32) >> 16
    return (bits[..., 0::2, :] | (bits[..., 1::2, :] << 16)).view(np.int32)


def _main_tile(j):
    if isinstance(j, int):
        return j if j < 2 else 2 if j < 4 else 3 if j < 8 else 4
    return jnp.where(j < 2, j, jnp.where(j < 4, 2, jnp.where(j < 8, 3, 4)))


def _constants():
    lag_val = _round_bf16(np.arange(S)).astype(np.int64)
    lane = np.arange(128)
    i, a = 4 * (lane // 16) + 2 * (lane % 2) + (lane // 8) % 2, (lane // 2) % 4
    first = np.array([[1, 3, 2, 4], [5, 7, 6, 8], [258, 260, 262, 264],
                      [516, 520, 772, 776], [1032, 1288, 1544, 1800]])
    lval = first[:, a] + 8 * i[None, :]
    lo = np.concatenate([lval[0, :64], lval[1, :64]])
    hi = np.concatenate([lval[0, 64:], lval[1, 64:]])
    lval[0], lval[1] = lo, hi
    where = {int(v): (t, p) for t in range(5) for p, v in enumerate(lval[t])}
    theta = np.pi * (4 * np.arange(T) + 1) / (2 * T)
    mats, extras = [], []
    for j in range(NC):
        per_tile = {}
        for m in range(1, T + 1):
            lag = T * j + m
            if lag >= S:
                continue
            t, p = where[int(lag_val[lag])]
            f = per_tile.setdefault(t, np.zeros((2 * T, 128)))
            f[:T, p] += np.cos(theta * m)
            f[T:, p] += np.sin(theta * m)
        main = _main_tile(j)
        mats.append(per_tile.pop(main))
        extras += [(j, t, f) for t, f in per_tile.items()]
    pairs = [(j, t, NC + n) for n, (j, t, _) in enumerate(extras)]
    mats += [f for _, _, f in extras]
    ang = theta[:, None] * np.arange(T)[None, :]
    fu = np.concatenate([np.cos(ang), np.sin(ang)], axis=0)
    mats.append(fu)
    row = np.arange(2 * T)
    ginv = fu.T[:, row // 16 * 16 + row % 2 * 8 + row % 16 // 2] / T
    return _pack_rows(np.stack(mats)), _pack_rows(ginv), pairs


_FMATS, _GINV, _EXTRAS = _constants()
_FU = _FMATS.shape[0] - 1


def _cmul(a, b):
    return a[0] * b[0] - a[1] * b[1], a[0] * b[1] + a[1] * b[0]


def _csq(a):
    return (a[0] + a[1]) * (a[0] - a[1]), (a[0] + a[0]) * a[1]


def _pack(even, odd):
    return pltpu.pack_elementwise([even, odd], packed_dtype=BF16).astype(jnp.int32)


def _halves(v):
    return pltpu.bitcast(v, BF16)


def _mult(v, n):
    return v if isinstance(v, int) else pl.multiple_of(v, n)


def _interleave(*streams):
    order = sorted((((n + 0.5) / len(st), k, n) for k, st in enumerate(streams) for n in range(len(st))))
    for _, k, n in order:
        streams[k][n]()


class _Pacer:
    def __init__(self, zero_ref, loads=True):
        self.ref, self.chain, self.loads = zero_ref, [zero_ref[0]], loads

    def __call__(self, hops):
        hops = int(hops * (1 if self.loads else HOPX))
        while len(self.chain) <= hops:
            last = self.chain[-1]
            self.chain.append(self.ref[last] if self.loads else last * last)
        return self.chain[hops]


def _iota(shape, axis):
    return jax.lax.broadcasted_iota(jnp.int32, shape, axis)


def _kernel(x_hbm, w_hbm, wo_hbm, are_hbm, aim_hbm, bre_hbm, bim_hbm, cre_hbm, cim_hbm,
            ldt_ref, dsk_ref, gw_ref, fm_hbm, gi_hbm, out_hbm,
            x_v, w_v, wo_v, par_v, fm_v, gi_v, row_v, lam_v, skip_v, st_v, wp_v, wk_v, wop_v,
            qkv_v, pt0_v, pt1_v, qt0_v, qt1_v, sd0_v, sd1_v, sd2_v, sd3_v, tmp0_v, tmp1_v, hold_v, zero_s, o_v, g_v, kc_v, u_v, kf0_v, kf1_v, kx_v, z_v, out_v, sems, osems):
    kf_v, pt_v, qt_v = (kf0_v, kf1_v), (pt0_v, pt1_v), (qt0_v, qt1_v)
    seed_v = (sd0_v, sd1_v, sd2_v, sd3_v)
    par_hbm = (are_hbm, aim_hbm, bre_hbm, bim_hbm, cre_hbm, cim_hbm)
    srcs = [(ref.at[:, 0:128], par_v.at[n, :, 0:128]) for n, ref in enumerate(par_hbm)]
    srcs += [(ref.at[:, 128:D], par_v.at[n, :, 128:D]) for n, ref in enumerate(par_hbm)]
    srcs += [(fm_hbm.at[_FU], fm_v.at[_FU]), (x_hbm, x_v), (fm_hbm.at[0:_FU], fm_v.at[0:_FU])]
    srcs += [(w_hbm.at[:, m * D:(m + 1) * D], w_v.at[m]) for m in range(3)]
    srcs += [(wo_hbm, wo_v), (gi_hbm, gi_v)]
    cps = [pltpu.make_async_copy(s, d, sems.at[n]) for n, (s, d) in enumerate(srcs)]
    cp_first, cp_par, cp_x, cp_rest = cps[:6], cps[6:12], cps[12:14], cps[14:]
    for cp in cp_first:
        cp.start()

    def discretise(c):
        cols = pl.ds(_mult(c * 128, 128), 128)
        dt = jnp.exp(row_v[0, c, 0:1, :]).astype(BF16).astype(F32)
        par = lambda p: par_v[p, :, cols].astype(F32)
        mag, ph = jnp.exp(dt * par(0)), dt * par(1)
        cr, ci = _cmul((par(4), par(5)), (dt * par(2), dt * par(3)))
        skip_v[c] = row_v[1, c] + jnp.sum(cr, axis=0, keepdims=True)
        for p, val in enumerate((mag * jnp.cos(ph), mag * jnp.sin(ph), cr, ci)):
            lam_v[p, cols, :] = val[0:128].T
            lam_v[4 + p, cols, :] = jnp.concatenate([val[128:N], val[128:N]], axis=0).T

    def power_tables(slot, k, r0, pace, h0):
        lane8, sub8 = _iota((8, 128), 1), _iota((8, 128), 0)
        low_rows, low_half = sub8 < 4, lane8 < 64
        sign_half = jnp.where(low_half, -1.0, 1.0).astype(F32)
        rows = pl.ds(r0 + k + pace(h0), 8, stride=4)
        pick = lambda p: [(lam_v[p, rows, :], lam_v[p + 1, rows, :]),
                          (lam_v[p + 4, rows, :], lam_v[p + 5, rows, :])]
        pw, c = {1: pick(0)}, pick(2)
        for e in range(9):
            pw[2 << e] = [_csq(v) for v in pw[1 << e]]
        mul = lambda a, b: [_cmul(u, v) for u, v in zip(a, b)]
        c1 = mul(c, pw[1])
        c2 = mul(c1, pw[1])
        c258 = mul(c2, pw[256])
        c262 = mul(c258, pw[4])
        p516 = mul(pw[4], pw[512])
        c516 = mul(c, p516)
        c772 = mul(c516, pw[256])
        c1032 = mul(c516, p516)
        c1544 = mul(c1032, pw[512])
        conj = lambda a: [(v[0], -v[1]) for v in a]
        one = [(jnp.ones((8, 128), F32), jnp.zeros((8, 128), F32))] * 2

        def split(top, bottom):
            return ([jnp.where(low_rows, u, pltpu.roll(v, 4, 0)) for u, v in zip(top, bottom)],
                    [jnp.where(low_rows, pltpu.roll(u, 4, 0), v) for u, v in zip(top, bottom)])

        def state(a, b):
            form = lambda v: (v[0][0], v[0][1], jnp.where(low_half, v[1][0], v[1][1]),
                              jnp.where(low_half, v[1][1], v[1][0]))
            return split(form(a), form(b))

        def factor(a):
            vals = (a[0][0], a[0][1], a[1][0], a[1][1] * sign_half)
            return split(vals, vals)

        def recur(a):
            vals = [v[0] + v[0] for v in a] + [v[0] * v[0] + v[1] * v[1] for v in a]
            return split(vals, vals)

        times = lambda s, m: _cmul(s, m) + (s[2] * m[2] + s[3] * m[3],)
        ahead = lambda x1, x0, r: (r[0] * x1[0] - r[2] * x0[0], r[0] * x1[1] - r[2] * x0[1],
                                   r[1] * x1[2] - r[3] * x0[2])
        def emit(ref, grp, tab):
            for n in range(0, len(tab), 2):
                for part in range(3):
                    ref[slot][4 * grp + k, 4 * n:4 * n + 8, part * 128:(part + 1) * 128] = _pack(
                        tab[n][part], tab[n + 1][part])

        q_seeds = [state(one, conj(pw[8])), factor(conj(pw[16])), recur(pw[16])]
        p_seeds = [state(c1, c2), state(c258, c262), state(c516, c772), state(c1032, c1544),
                   factor(pw[2]), factor(pw[4]), factor(pw[256]), recur(pw[2])]
        zero = [pl.ds(_mult(pace(h0 + (PF[0] + PF[1] * grp) * H1), 8), 8) for grp in range(2)]
        for grp in range(2):
            s0, s2, s3, s4, m2, m4, m256, r2 = [v[grp] for v in p_seeds]
            p_rows = [s0, times(s0, m2)]
            for _ in range(2):
                p_rows.append(ahead(p_rows[-1], p_rows[-2], r2))
            p_rows += [s2, times(s2, m2), s3, times(s3, m4), s4, times(s4, m256)]
            emit(pt_v, grp, p_rows)
            for n, v in enumerate(x for sd in q_seeds for x in sd[grp]):
                seed_v[k][grp, n] = v
        for grp in range(2):
            q0, m16, r16 = [[seed_v[k][grp, 4 * w + n, zero[grp], :] for n in range(4)] for w in range(3)]
            q_rows = [q0, times(q0, m16)]
            for _ in range(14):
                q_rows.append(ahead(q_rows[-1], q_rows[-2], r16))
            emit(qt_v, grp, q_rows)

    def taps16(slot, grp, r0):
        lane8, sub8 = _iota((8, 128), 1), _iota((8, 128), 0)
        diag = ((lane8 >> 1) & 3) == (sub8 >> 1)
        shift = (sub8 & 1) - (sub8 >> 1)
        own = []
        for k in range(4):
            out = jax.lax.dot_general(_halves(pt_v[slot][4 * grp + k]), _halves(qt_v[slot][4 * grp + k]),
                                      NT_DIMS, preferred_element_type=F32)
            tiles = []
            for t in range(5):
                n = jnp.where(diag, out[16 * t:16 * t + 8], pltpu.roll(out[16 * t + 8:16 * t + 16], 4, 1))
                val = n
                for d in (1, -1, -2, -3):
                    val = jnp.where(shift == d, pltpu.roll(n, (2 * d) % 128, 1), val)
                tiles.append(val)
            own.append(tiles)
        low_res, even_row, low_half = (lane8 & 2) == 0, (sub8 & 1) == 0, lane8 < 64
        halves = []
        for k in range(2):
            res = [jnp.where(even_row, jnp.where(low_res, a, pltpu.roll(a, 7, 0)),
                             jnp.where(low_res, pltpu.roll(b, 1, 0), b)) for a, b in zip(own[k], own[k + 2])]
            res[0], res[1] = (jnp.where(low_half, res[0], pltpu.roll(res[1], 64, 1)),
                              jnp.where(low_half, pltpu.roll(res[0], 64, 1), res[1]))
            halves.append(res)
        for t in range(5):
            kc_v[t, pl.ds(_mult(r0 // 2, 8), 8), :] = _pack(halves[0][t], halves[1][t])

    def gather_heads(st, dst, row0, cols):
        for d in range(DH):
            for h in range(0, H, 16):
                even, odd = [st[pl.ds((h + e) * DH + d, 8, stride=2 * DH), :] for e in range(2)]
                dst[pl.ds(row0 + (d * H + h) // 2, 8), cols] = _pack(even, odd)

    def permute_w(m, kt):
        cols = pl.ds(_mult(kt * 128, 128), 128)
        for n in range(CT):
            st_v[m, n * 128:(n + 1) * 128, :] = w_v[m, cols, n * 128:(n + 1) * 128].astype(F32).T
        gather_heads(st_v.at[m], wk_v if m == 1 else wp_v, 0 if m == 1 else m * D // 4, cols)

    def permute_wo(c):
        cols = pl.ds(_mult(c * 128, 128), 128)
        st_v[1] = wo_v[:, cols].astype(F32)
        gather_heads(st_v.at[1], wop_v, 0, cols)

    def proj_tile(m, c, r0, nrows):
        src, tile = (wk_v, c) if isinstance(m, int) and m == 1 else (wp_v, m // 2 * CT + c)
        wt = _halves(src[pl.ds(_mult(tile * 64, 64), 64), :])
        res = jax.lax.dot_general(x_v[pl.ds(r0, nrows), :], wt, NT_DIMS, preferred_element_type=F32)
        qkv_v[m * CT + c, pl.ds(r0 + HALO, nrows), :] = res

    def gate(r0, nrows):
        xf = x_v[pl.ds(r0, nrows), :].astype(F32)
        z = functools.reduce(lambda a, b: a + b,
                             [xf[:, c * 128:(c + 1) * 128] * row_v[2, c, 0:1, :] for c in range(CT)])
        z = jnp.sum(z, axis=1, keepdims=True)
        g_v[pl.ds(r0, nrows), :] = jnp.broadcast_to(0.5 * jnp.tanh(0.5 * z) + 0.5, (nrows, 128))

    def udft(c, j):
        xs = x_v[pl.ds(_mult(j * T, T), T), pl.ds(_mult(c * 128, 128), 128)]
        u_v[c, j] = jnp.dot(_halves(fm_v[_FU]), xs, preferred_element_type=F32)

    def attn_rows(r0, nrows, masked, pace, h0, dst):
        at = lambda h: r0 + HALO + pace(h0 + h)

        def taps(plane, base, r):
            strip = qkv_v[plane, pl.ds(base - DIL * r - 8, nrows + 8), :]
            return strip[8:], strip[:nrows]

        q = [qkv_v[c, pl.ds(at(0), nrows), :] for c in range(CT)]
        logits = [None] * WIN
        for r in range(WIN // 2):
            base = at(r * H3_W)
            ks = [taps(CT + c, base, r) for c in range(CT)]
            for e in range(2):
                w = r + e * (WIN // 2)
                s = functools.reduce(lambda a, b: a + b, [q[c] * ks[c][e] for c in range(CT)])
                s = s + pltpu.roll(s, 64, 1)
                s = s + pltpu.roll(s, 32, 1)
                if masked and w > 0:
                    s = jnp.where(r0 + _iota((nrows, 128), 0) >= DIL * w, s, -1e9 * DH ** 0.5)
                logits[w] = s
        top = functools.reduce(jnp.maximum, logits)
        p = [jnp.exp2((s - top) * (DH ** -0.5 * LOG2E)) for s in logits]
        den = functools.reduce(lambda a, b: a + b, p)
        inv = pl.reciprocal(den, approx=True)
        inv = inv * (2.0 - den * inv)
        for c in range(CT):
            base = at(H3_LATE + c * H3_C)
            acc = None
            for r in range(WIN // 2):
                near, far = taps(2 * CT + c, base, r)
                part = p[r] * near + p[r + WIN // 2] * far
                acc = part if acc is None else acc + part
            dst[:, c * 128:(c + 1) * 128] = pltpu.bitcast(
                (acc * inv).astype(BF16), jnp.int32)

    def spectrum(c, t, n):
        taps = _halves(kc_v[t, c * 64:(c + 1) * 64, :])
        return jax.lax.dot_general(_halves(fm_v[n]), taps, NT_DIMS, preferred_element_type=F32)

    def kdft(c, j):
        taps = _halves(kc_v[_main_tile(j), c * 64:(c + 1) * 64, :])
        for e in range(2 * T // MK):
            kf_v[c % 2][j, e * MK:(e + 1) * MK, :] = jax.lax.dot_general(
                _halves(fm_v[j, e * MK // 2:(e + 1) * MK // 2, :]), taps, NT_DIMS, preferred_element_type=F32)

    def kdft_extra(c, n):
        kx_v[c, n] = spectrum(c, _EXTRAS[n][1], _EXTRAS[n][2])

    def conv(c, fb, tmp, pace, h0, dh, put):
        def rows(k):
            r = fb * 8 + pace(h0 + k * dh / 100)
            return pl.ds(_mult(r, 8), 8), pl.ds(_mult(r + T, 8), 8)

        re, im = rows(0)
        kr = [kf_v[c % 2][j, re, :] for j in range(NC)]
        ki = [kf_v[c % 2][j, im, :] for j in range(NC)]
        kr[0] = kr[0] + skip_v[c]
        for n, (j, _, _) in enumerate(_EXTRAS):
            kr[j] = kr[j] + kx_v[c, n, re, :]
            ki[j] = ki[j] + kx_v[c, n, im, :]
        kr, ki = ([kr[0]] + [kr[j] + ki[j - 1] for j in range(1, NC)],
                  [ki[0]] + [ki[j] - kr[j - 1] for j in range(1, NC)])
        half = NC // 2
        for part, k in enumerate((kr, ki)):
            for a in range(half):
                tmp[2 * part, a] = k[2 * a]
                tmp[2 * part, half + a] = (k[2 * a - 1] if a else 0.0) - k[2 * a]
                tmp[2 * part + 1, a] = k[2 * a + 1] - k[2 * a]

        def toeplitz(a, b):
            return [functools.reduce(lambda x, y: x + y, [a[j] * b[i - j] for j in range(i + 1)])
                    for i in range(half)]

        for n in range(3):
            done = 60 + n * PER_PRODUCT
            re, im = rows(done)
            zero = pl.ds(_mult(pace(h0 + done * dh / 100), 8), 8)
            ar, ai = [[tmp[2 * part + n // 2, n % 2 * half + a, zero, :] for a in range(half)] for part in range(2)]
            chunks = lambda e: [[u_v[c, 2 * b + e, r, :] for b in range(half)] for r in (re, im)]
            if n == 0:
                ur, ui = [[x + y for x, y in zip(p, q)] for p, q in zip(chunks(0), chunks(1))]
            else:
                ur, ui = chunks(2 - n)
            k1 = toeplitz(ar, [x + y for x, y in zip(ur, ui)])
            k3 = toeplitz([x + y for x, y in zip(ar, ai)], ui)
            k2 = toeplitz([y - x for x, y in zip(ar, ai)], ur)
            for i in range(half):
                for part, val in enumerate((k1[i] - k3[i], k1[i] + k2[i])):
                    if n == 0:
                        tmp[2 * part + 1, half + i] = val
                    else:
                        put(part, 2 * i + n - 1, tmp[2 * part + 1, half + i] + val)

    def conv_pair(c, s, n, pace, h0, dh):
        def hold(part, i, val):
            hold_v[2 * n + part, i] = val

        def store(part, i, val):
            rows = pl.ds(_mult(part * (T // 2) + s * 8, 8), 8)
            z_v[i, rows, c * 128:(c + 1) * 128] = _pack(hold_v[2 * n + part, i], val)

        conv(c, 2 * s, tmp0_v, pace, h0, dh, hold)
        conv(c, 2 * s + 1, tmp1_v, pace, h0 + 8.1 * dh, dh, store)

    def finish_chunk(i, slot):
        a = jnp.dot(_halves(o_v[slot]), _halves(wop_v[...]),
                    preferred_element_type=F32)
        for n in range(AB // T):
            rows = pl.ds(_mult(i * AB + n * T, T), T)
            y = jnp.dot(_halves(gi_v[...]), _halves(z_v[i * (AB // T) + n]), preferred_element_type=F32)
            g = g_v[rows, :]
            for c in range(CT):
                cols = slice(c * 128, (c + 1) * 128)
                mixed = y[:, cols] + g * (a[n * T:(n + 1) * T, cols] - y[:, cols])
                out_v[rows, cols] = mixed.astype(out_v.dtype)

    def out_copy(i):
        rows = pl.ds(_mult(i * AB, AB), AB)
        return pltpu.make_async_copy(out_v.at[rows], out_hbm.at[rows], osems.at[i])

    def loop(n, body):
        jax.lax.fori_loop(0, n, lambda it, _: body(it), None)

    for p, ref in enumerate((ldt_ref, dsk_ref, gw_ref)):
        vec = ref[...].astype(F32).reshape(1, D)
        for c in range(CT):
            row_v[p, c] = jnp.broadcast_to(vec[:, c * 128:(c + 1) * 128], (8, 128))
    zero_s[0] = 0
    for cp in cp_first:
        cp.wait()
    for cp in cp_par:
        cp.start()

    def discretise_step(c):
        @pl.when(c == 1)
        def _():
            for cp in cp_par:
                cp.wait()
            for cp in cp_x:
                cp.start()

        discretise(c)

    loop(CT, discretise_step)
    for n in range(CT, 3 * CT):
        qkv_v[n, 0:HALO, :] = jnp.zeros((HALO, 128), F32)
    P = functools.partial

    def tables(b, slot, pace, h0):
        for k in range(4):
            power_tables(slot, k, b * 32, pace, h0 + H1 * k)

    def taps(b, slot):
        for n in range(2):
            taps16(slot, n, b * 32 + n * 16)

    def key_units(b):
        for u in (2 * b, 2 * b + 1):
            s, c = u // CT, u % CT
            for e in range(RB // T):
                udft(c, s * (RB // T) + e)
            gate(_mult(s * RB + jnp.minimum(c, 3) * (RB // 4), RB // 4), RB // 4)

    def phase1(it):
        pace = _Pacer(zero_s)
        taps(2 * it, 0)
        key_units(2 * it)
        tables(2 * it + 1, 1, pace, 0)
        key_units(2 * it + 1)
        taps(2 * it + 1, 1)
        tables(jnp.minimum(2 * it + 2, n1 - 1), 0, pace, 4 * H1)

    n1 = D // 32
    tables(0, 0, lambda h: 0, 0)
    for cp in cp_x:
        cp.wait()
    for cp in cp_rest:
        cp.start()
    loop(n1 // 2, phase1)

    for cp in cp_rest:
        cp.wait()
    _interleave([P(kdft, 0, j) for j in range(NC)]
                + [P(kdft_extra, c, n) for c in range(CT) for n in range(len(_EXTRAS))],
                [P(permute_w, 1, kt) for kt in range(CT)])

    def keys(c):
        proj_tile(1, c, 0, S)
        permute_w(0, c)
        permute_w(2, c)
        permute_wo(c)

    loop(CT, keys)

    def qv_unit(u):
        s, r = u // (2 * CT), u % (2 * CT)
        for e in range(RB // MR):
            proj_tile(2 * (r // CT), r % CT, _mult(s * RB + e * MR, MR), MR)

    pairs = T // 16
    for c in range(CT):
        def phase2(it, c=c):
            pace = _Pacer(zero_s)
            for n in range(CP):
                s = it * CP + n
                if c + 1 < CT:
                    for e in range(2):
                        qv_unit(2 * (c * pairs + s) + e)
                        kdft(c + 1, 2 * s + e)
                else:
                    qv_unit(2 * c * pairs + s)
            dh = H2 if c + 1 < CT else H2_LAST
            for n in range(CP):
                conv_pair(c, it * CP + n, n, pace, n * 16.2 * dh, dh)

        loop(pairs // CP, phase2)

    def attn_chunk(i, slot, pace, gap):
        for n in range(AB // AR):
            attn_rows(_mult(i * AB + n * AR, AR), AR, isinstance(i, int) and i * AB + n * AR < HALO,
                      pace, n * gap, o_v.at[slot, n * AR // 2:(n + 1) * AR // 2])

    def phase3(i):
        pace = _Pacer(zero_s, loads=False)
        finish_chunk(i - 1, (i - 1) % 2)
        attn_chunk(i, i % 2, pace, H3)
        out_copy(i - 1).start()

    last = S // AB - 1
    for u in range((2 * CT - 1) * pairs, 2 * CT * pairs):
        qv_unit(u)
    attn_chunk(0, 0, _Pacer(zero_s), H3_FIRST)
    loop(last, lambda it: phase3(it + 1))
    finish_chunk(last, last % 2)
    out_copy(last).start()
    for i in range(last + 1):
        out_copy(i).wait()


@jax.jit
def pallas_gated_mix__sliding_local_dilated__ssm_conv_s4__prompt_kernel(
    A_x: jax.Array,
    A_wqkv: jax.Array,
    A_wo: jax.Array,
    B_u: jax.Array,
    B_A_re: jax.Array,
    B_A_im: jax.Array,
    B_B_re: jax.Array,
    B_B_im: jax.Array,
    B_C_re: jax.Array,
    B_C_im: jax.Array,
    B_log_dt: jax.Array,
    B_Dskip: jax.Array,
    gate_w: jax.Array,
):
    del B_u
    assert A_x.shape == (1, S, D) and B_A_re.shape == (D, N) and B_A_re.dtype == BF16
    hbm = pl.BlockSpec(memory_space=pl.ANY)
    vmem = pl.BlockSpec(memory_space=pltpu.VMEM)
    scratch = [
        pltpu.VMEM((S, D), BF16),
        pltpu.VMEM((3, D, D), BF16),
        pltpu.VMEM((D, D), BF16),
        pltpu.VMEM((6, N, D), BF16),
        pltpu.VMEM(_FMATS.shape, jnp.int32),
        pltpu.VMEM(_GINV.shape, jnp.int32),
        pltpu.VMEM((3, CT, 8, 128), F32),
        pltpu.VMEM((8, D, 128), F32),
        pltpu.VMEM((CT, 8, 128), F32),
        pltpu.VMEM((3, D, 128), F32),
        pltpu.VMEM((D, D), jnp.int32),
        pltpu.VMEM((D // 2, D), jnp.int32),
        pltpu.VMEM((D // 2, D), jnp.int32),
        pltpu.VMEM((3 * CT, S + HALO, 128), F32),
        pltpu.VMEM((8, 40, 3 * 128), jnp.int32),
        pltpu.VMEM((8, 40, 3 * 128), jnp.int32),
        pltpu.VMEM((8, 64, 3 * 128), jnp.int32),
        pltpu.VMEM((8, 64, 3 * 128), jnp.int32),
        *[pltpu.VMEM((2, 12, 8, 128), F32)] * 4,
        pltpu.VMEM((4, NC, 8, 128), F32),
        pltpu.VMEM((4, NC, 8, 128), F32),
        pltpu.VMEM((2 * CP, NC, 8, 128), F32),
        pltpu.SMEM((1,), jnp.int32),
        pltpu.VMEM((2, AB // 2, D), jnp.int32),
        pltpu.VMEM((S, 128), F32),
        pltpu.VMEM((5, D // 2, 128), jnp.int32),
        pltpu.VMEM((CT, NC, 2 * T, 128), F32),
        pltpu.VMEM((NC, 2 * T, 128), F32),
        pltpu.VMEM((NC, 2 * T, 128), F32),
        pltpu.VMEM((CT, len(_EXTRAS), 2 * T, 128), F32),
        pltpu.VMEM((NC, T, D), jnp.int32),
        pltpu.VMEM((S, D), BF16),
        pltpu.SemaphoreType.DMA((20,)),
        pltpu.SemaphoreType.DMA((NC,)),
    ]
    out = pl.pallas_call(
        _kernel,
        out_shape=jax.ShapeDtypeStruct((S, D), A_x.dtype),
        in_specs=[hbm] * 9 + [vmem] * 3 + [hbm] * 2,
        out_specs=hbm,
        scratch_shapes=scratch,
        compiler_params=pltpu.CompilerParams(vmem_limit_bytes=100 * 1024 * 1024),
    )(A_x.reshape(S, D), A_wqkv, A_wo, B_A_re.T, B_A_im.T, B_B_re.T, B_B_im.T, B_C_re.T, B_C_im.T,
      B_log_dt, B_Dskip, gate_w, _FMATS, _GINV)
    return out.reshape(1, S, D)
```

```python
import functools

import jax
import jax.numpy as jnp
import numpy as np
import jax.experimental.pallas as pl
import jax.experimental.pallas.tpu as pltpu

S = 2048
D = 640
N = 192
H = 32
DH = D // H
WIN, DIL = 8, 2
HALO = 16
T = 128
NC = S // T
CT = D // 128
F32, BF16 = jnp.float32, jnp.bfloat16
RB = 256
MR = 128
MK = 128
MU = 128
MO = 256
AB = 256
AR = 16
CP = 4
HOPX, PF, PER_PRODUCT = 3, (0.6, 0.5), 250
H1, H2, H2_LAST = 27, 8, 6
H3, H3_W, H3_C, H3_LATE, H3_FIRST = 20, 3, 3, 56, 24
LOG2E = 1.4426950408889634
NT_DIMS = (((1,), (1,)), ((), ()))


def _round_bf16(v):
    u = np.asarray(v, np.float32).view(np.uint32)
    u = (u + 0x7FFF + ((u >> 16) & 1)) & 0xFFFF0000
    return u.view(np.float32)


def _pack_rows(m):
    bits = np.ascontiguousarray(_round_bf16(m)).view(np.uint32) >> 16
    return (bits[..., 0::2, :] | (bits[..., 1::2, :] << 16)).view(np.int32)


def _main_tile(j):
    if isinstance(j, int):
        return j if j < 2 else 2 if j < 4 else 3 if j < 8 else 4
    return jnp.where(j < 2, j, jnp.where(j < 4, 2, jnp.where(j < 8, 3, 4)))


def _constants():
    lag_val = _round_bf16(np.arange(S)).astype(np.int64)
    lane = np.arange(128)
    i, a = 4 * (lane // 16) + 2 * (lane % 2) + (lane // 8) % 2, (lane // 2) % 4
    first = np.array([[1, 3, 2, 4], [5, 7, 6, 8], [258, 260, 262, 264],
                      [516, 520, 772, 776], [1032, 1288, 1544, 1800]])
    lval = first[:, a] + 8 * i[None, :]
    lo = np.concatenate([lval[0, :64], lval[1, :64]])
    hi = np.concatenate([lval[0, 64:], lval[1, 64:]])
    lval[0], lval[1] = lo, hi
    where = {int(v): (t, p) for t in range(5) for p, v in enumerate(lval[t])}
    theta = np.pi * (4 * np.arange(T) + 1) / (2 * T)
    mats, extras = [], []
    for j in range(NC):
        per_tile = {}
        for m in range(1, T + 1):
            lag = T * j + m
            if lag >= S:
                continue
            t, p = where[int(lag_val[lag])]
            f = per_tile.setdefault(t, np.zeros((2 * T, 128)))
            f[:T, p] += np.cos(theta * m)
            f[T:, p] += np.sin(theta * m)
        main = _main_tile(j)
        mats.append(per_tile.pop(main))
        extras += [(j, t, f) for t, f in per_tile.items()]
    pairs = [(j, t, NC + n) for n, (j, t, _) in enumerate(extras)]
    mats += [f for _, _, f in extras]
    ang = theta[:, None] * np.arange(T)[None, :]
    fu = np.concatenate([np.cos(ang), np.sin(ang)], axis=0)
    mats.append(fu)
    row = np.arange(2 * T)
    ginv = fu.T[:, row // 16 * 16 + row % 2 * 8 + row % 16 // 2] / T
    return _pack_rows(np.stack(mats)), _pack_rows(ginv), pairs


_FMATS, _GINV, _EXTRAS = _constants()
_FU = _FMATS.shape[0] - 1


def _cmul(a, b):
    return a[0] * b[0] - a[1] * b[1], a[0] * b[1] + a[1] * b[0]


def _csq(a):
    return (a[0] + a[1]) * (a[0] - a[1]), (a[0] + a[0]) * a[1]


def _pack(even, odd):
    return pltpu.pack_elementwise([even, odd], packed_dtype=BF16).astype(jnp.int32)


def _halves(v):
    return pltpu.bitcast(v, BF16)


def _mult(v, n):
    return v if isinstance(v, int) else pl.multiple_of(v, n)


def _interleave(*streams):
    order = sorted((((n + 0.5) / len(st), k, n) for k, st in enumerate(streams) for n in range(len(st))))
    for _, k, n in order:
        streams[k][n]()


class _Pacer:
    def __init__(self, zero_ref, loads=True):
        self.ref, self.chain, self.loads = zero_ref, [zero_ref[0]], loads

    def __call__(self, hops):
        hops = int(hops * (1 if self.loads else HOPX))
        while len(self.chain) <= hops:
            last = self.chain[-1]
            self.chain.append(self.ref[last] if self.loads else last * last)
        return self.chain[hops]


def _iota(shape, axis):
    return jax.lax.broadcasted_iota(jnp.int32, shape, axis)


def _kernel(x_hbm, w_hbm, wo_hbm, are_hbm, aim_hbm, bre_hbm, bim_hbm, cre_hbm, cim_hbm,
            ldt_ref, dsk_ref, gw_ref, fm_hbm, gi_hbm, out_hbm,
            x_v, w_v, wo_v, par_v, fm_v, gi_v, row_v, lam_v, skip_v, st_v, wp_v, wk_v, wop_v,
            qkv_v, pt0_v, pt1_v, qt0_v, qt1_v, sd0_v, sd1_v, sd2_v, sd3_v, tmp0_v, tmp1_v, hold_v, zero_s, o_v, g_v, kc_v, u_v, kf0_v, kf1_v, kx_v, z_v, out_v, sems, osems):
    kf_v, pt_v, qt_v = (kf0_v, kf1_v), (pt0_v, pt1_v), (qt0_v, qt1_v)
    seed_v = (sd0_v, sd1_v, sd2_v, sd3_v)
    par_hbm = (are_hbm, aim_hbm, bre_hbm, bim_hbm, cre_hbm, cim_hbm)
    srcs = [(ref.at[:, 0:128], par_v.at[n, :, 0:128]) for n, ref in enumerate(par_hbm)]
    srcs += [(ref.at[:, 128:D], par_v.at[n, :, 128:D]) for n, ref in enumerate(par_hbm)]
    srcs += [(fm_hbm.at[_FU], fm_v.at[_FU]), (x_hbm, x_v), (fm_hbm.at[0:_FU], fm_v.at[0:_FU])]
    srcs += [(w_hbm.at[:, m * D:(m + 1) * D], w_v.at[m]) for m in range(3)]
    srcs += [(wo_hbm, wo_v), (gi_hbm, gi_v)]
    cps = [pltpu.make_async_copy(s, d, sems.at[n]) for n, (s, d) in enumerate(srcs)]
    cp_first, cp_par, cp_x, cp_rest = cps[:6], cps[6:12], cps[12:14], cps[14:]
    for cp in cp_first:
        cp.start()

    def discretise(c):
        cols = pl.ds(_mult(c * 128, 128), 128)
        dt = jnp.exp(row_v[0, c, 0:1, :]).astype(BF16).astype(F32)
        par = lambda p: par_v[p, :, cols].astype(F32)
        mag, ph = jnp.exp(dt * par(0)), dt * par(1)
        cr, ci = _cmul((par(4), par(5)), (dt * par(2), dt * par(3)))
        skip_v[c] = row_v[1, c] + jnp.sum(cr, axis=0, keepdims=True)
        for p, val in enumerate((mag * jnp.cos(ph), mag * jnp.sin(ph), cr, ci)):
            lam_v[p, cols, :] = val[0:128].T
            lam_v[4 + p, cols, :] = jnp.concatenate([val[128:N], val[128:N]], axis=0).T

    def power_tables(slot, k, r0, pace, h0):
        lane8, sub8 = _iota((8, 128), 1), _iota((8, 128), 0)
        low_rows, low_half = sub8 < 4, lane8 < 64
        sign_half = jnp.where(low_half, -1.0, 1.0).astype(F32)
        rows = pl.ds(r0 + k + pace(h0), 8, stride=4)
        pick = lambda p: [(lam_v[p, rows, :], lam_v[p + 1, rows, :]),
                          (lam_v[p + 4, rows, :], lam_v[p + 5, rows, :])]
        pw, c = {1: pick(0)}, pick(2)
        for e in range(9):
            pw[2 << e] = [_csq(v) for v in pw[1 << e]]
        mul = lambda a, b: [_cmul(u, v) for u, v in zip(a, b)]
        c1 = mul(c, pw[1])
        c2 = mul(c1, pw[1])
        c258 = mul(c2, pw[256])
        c262 = mul(c258, pw[4])
        p516 = mul(pw[4], pw[512])
        c516 = mul(c, p516)
        c772 = mul(c516, pw[256])
        c1032 = mul(c516, p516)
        c1544 = mul(c1032, pw[512])
        conj = lambda a: [(v[0], -v[1]) for v in a]
        one = [(jnp.ones((8, 128), F32), jnp.zeros((8, 128), F32))] * 2

        def split(top, bottom):
            return ([jnp.where(low_rows, u, pltpu.roll(v, 4, 0)) for u, v in zip(top, bottom)],
                    [jnp.where(low_rows, pltpu.roll(u, 4, 0), v) for u, v in zip(top, bottom)])

        def state(a, b):
            form = lambda v: (v[0][0], v[0][1], jnp.where(low_half, v[1][0], v[1][1]),
                              jnp.where(low_half, v[1][1], v[1][0]))
            return split(form(a), form(b))

        def factor(a):
            vals = (a[0][0], a[0][1], a[1][0], a[1][1] * sign_half)
            return split(vals, vals)

        def recur(a):
            vals = [v[0] + v[0] for v in a] + [v[0] * v[0] + v[1] * v[1] for v in a]
            return split(vals, vals)

        times = lambda s, m: _cmul(s, m) + (s[2] * m[2] + s[3] * m[3],)
        ahead = lambda x1, x0, r: (r[0] * x1[0] - r[2] * x0[0], r[0] * x1[1] - r[2] * x0[1],
                                   r[1] * x1[2] - r[3] * x0[2])
        def emit(ref, grp, tab):
            for n in range(0, len(tab), 2):
                for part in range(3):
                    ref[slot][4 * grp + k, 4 * n:4 * n + 8, part * 128:(part + 1) * 128] = _pack(
                        tab[n][part], tab[n + 1][part])

        q_seeds = [state(one, conj(pw[8])), factor(conj(pw[16])), recur(pw[16])]
        p_seeds = [state(c1, c2), state(c258, c262), state(c516, c772), state(c1032, c1544),
                   factor(pw[2]), factor(pw[4]), factor(pw[256]), recur(pw[2])]
        zero = [pl.ds(_mult(pace(h0 + (PF[0] + PF[1] * grp) * H1), 8), 8) for grp in range(2)]
        for grp in range(2):
            s0, s2, s3, s4, m2, m4, m256, r2 = [v[grp] for v in p_seeds]
            p_rows = [s0, times(s0, m2)]
            for _ in range(2):
                p_rows.append(ahead(p_rows[-1], p_rows[-2], r2))
            p_rows += [s2, times(s2, m2), s3, times(s3, m4), s4, times(s4, m256)]
            emit(pt_v, grp, p_rows)
            for n, v in enumerate(x for sd in q_seeds for x in sd[grp]):
                seed_v[k][grp, n] = v
        for grp in range(2):
            q0, m16, r16 = [[seed_v[k][grp, 4 * w + n, zero[grp], :] for n in range(4)] for w in range(3)]
            q_rows = [q0, times(q0, m16)]
            for _ in range(14):
                q_rows.append(ahead(q_rows[-1], q_rows[-2], r16))
            emit(qt_v, grp, q_rows)

    def taps16(slot, grp, r0):
        lane8, sub8 = _iota((8, 128), 1), _iota((8, 128), 0)
        diag = ((lane8 >> 1) & 3) == (sub8 >> 1)
        shift = (sub8 & 1) - (sub8 >> 1)
        own = []
        for k in range(4):
            out = jax.lax.dot_general(_halves(pt_v[slot][4 * grp + k]), _halves(qt_v[slot][4 * grp + k]),
                                      NT_DIMS, preferred_element_type=F32)
            tiles = []
            for t in range(5):
                n = jnp.where(diag, out[16 * t:16 * t + 8], pltpu.roll(out[16 * t + 8:16 * t + 16], 4, 1))
                val = n
                for d in (1, -1, -2, -3):
                    val = jnp.where(shift == d, pltpu.roll(n, (2 * d) % 128, 1), val)
                tiles.append(val)
            own.append(tiles)
        low_res, even_row, low_half = (lane8 & 2) == 0, (sub8 & 1) == 0, lane8 < 64
        halves = []
        for k in range(2):
            res = [jnp.where(even_row, jnp.where(low_res, a, pltpu.roll(a, 7, 0)),
                             jnp.where(low_res, pltpu.roll(b, 1, 0), b)) for a, b in zip(own[k], own[k + 2])]
            res[0], res[1] = (jnp.where(low_half, res[0], pltpu.roll(res[1], 64, 1)),
                              jnp.where(low_half, pltpu.roll(res[0], 64, 1), res[1]))
            halves.append(res)
        for t in range(5):
            kc_v[t, pl.ds(_mult(r0 // 2, 8), 8), :] = _pack(halves[0][t], halves[1][t])

    def gather_heads(st, dst, row0, cols):
        for d in range(DH):
            for h in range(0, H, 16):
                even, odd = [st[pl.ds((h + e) * DH + d, 8, stride=2 * DH), :] for e in range(2)]
                dst[pl.ds(row0 + (d * H + h) // 2, 8), cols] = _pack(even, odd)

    def permute_w(m, kt):
        cols = pl.ds(_mult(kt * 128, 128), 128)
        for n in range(CT):
            st_v[m, n * 128:(n + 1) * 128, :] = w_v[m, cols, n * 128:(n + 1) * 128].astype(F32).T
        gather_heads(st_v.at[m], wk_v if m == 1 else wp_v, 0 if m == 1 else m * D // 4, cols)

    def permute_wo(c):
        cols = pl.ds(_mult(c * 128, 128), 128)
        st_v[1] = wo_v[:, cols].astype(F32)
        gather_heads(st_v.at[1], wop_v, 0, cols)

    def proj_tile(m, c, r0, nrows):
        src, tile = (wk_v, c) if isinstance(m, int) and m == 1 else (wp_v, m // 2 * CT + c)
        wt = _halves(src[pl.ds(_mult(tile * 64, 64), 64), :])
        res = jax.lax.dot_general(x_v[pl.ds(r0, nrows), :], wt, NT_DIMS, preferred_element_type=F32)
        qkv_v[m * CT + c, pl.ds(r0 + HALO, nrows), :] = res

    def gate(r0, nrows):
        xf = x_v[pl.ds(r0, nrows), :].astype(F32)
        z = functools.reduce(lambda a, b: a + b,
                             [xf[:, c * 128:(c + 1) * 128] * row_v[2, c, 0:1, :] for c in range(CT)])
        z = jnp.sum(z, axis=1, keepdims=True)
        g_v[pl.ds(r0, nrows), :] = jnp.broadcast_to(0.5 * jnp.tanh(0.5 * z) + 0.5, (nrows, 128))

    def udft(c, j):
        xs = x_v[pl.ds(_mult(j * T, T), T), pl.ds(_mult(c * 128, 128), 128)]
        for e in range(2 * T // MU):
            u_v[c, j, e * MU:(e + 1) * MU, :] = jnp.dot(
                _halves(fm_v[_FU, e * MU // 2:(e + 1) * MU // 2, :]), xs, preferred_element_type=F32)

    def attn_rows(r0, nrows, masked, pace, h0, dst):
        at = lambda h: r0 + HALO + pace(h0 + h)

        def taps(plane, base, r):
            strip = qkv_v[plane, pl.ds(base - DIL * r - 8, nrows + 8), :]
            return strip[8:], strip[:nrows]

        q = [qkv_v[c, pl.ds(at(0), nrows), :] for c in range(CT)]
        logits = [None] * WIN
        for r in range(WIN // 2):
            base = at(r * H3_W)
            ks = [taps(CT + c, base, r) for c in range(CT)]
            for e in range(2):
                w = r + e * (WIN // 2)
                s = functools.reduce(lambda a, b: a + b, [q[c] * ks[c][e] for c in range(CT)])
                s = s + pltpu.roll(s, 64, 1)
                s = s + pltpu.roll(s, 32, 1)
                if masked and w > 0:
                    s = jnp.where(r0 + _iota((nrows, 128), 0) >= DIL * w, s, -1e9 * DH ** 0.5)
                logits[w] = s
        top = functools.reduce(jnp.maximum, logits)
        p = [jnp.exp2((s - top) * (DH ** -0.5 * LOG2E)) for s in logits]
        den = functools.reduce(lambda a, b: a + b, p)
        inv = pl.reciprocal(den, approx=True)
        inv = inv * (2.0 - den * inv)
        for c in range(CT):
            base = at(H3_LATE + c * H3_C)
            acc = None
            for r in range(WIN // 2):
                near, far = taps(2 * CT + c, base, r)
                part = p[r] * near + p[r + WIN // 2] * far
                acc = part if acc is None else acc + part
            dst[:, c * 128:(c + 1) * 128] = pltpu.bitcast(
                (acc * inv).astype(BF16), jnp.int32)

    def spectrum(c, t, n):
        taps = _halves(kc_v[t, c * 64:(c + 1) * 64, :])
        return jax.lax.dot_general(_halves(fm_v[n]), taps, NT_DIMS, preferred_element_type=F32)

    def kdft(c, j):
        taps = _halves(kc_v[_main_tile(j), c * 64:(c + 1) * 64, :])
        for e in range(2 * T // MK):
            kf_v[c % 2][j, e * MK:(e + 1) * MK, :] = jax.lax.dot_general(
                _halves(fm_v[j, e * MK // 2:(e + 1) * MK // 2, :]), taps, NT_DIMS, preferred_element_type=F32)

    def kdft_extra(c, n):
        kx_v[c, n] = spectrum(c, _EXTRAS[n][1], _EXTRAS[n][2])

    def conv(c, fb, tmp, pace, h0, dh, put):
        def rows(k):
            r = fb * 8 + pace(h0 + k * dh / 100)
            return pl.ds(_mult(r, 8), 8), pl.ds(_mult(r + T, 8), 8)

        re, im = rows(0)
        kr = [kf_v[c % 2][j, re, :] for j in range(NC)]
        ki = [kf_v[c % 2][j, im, :] for j in range(NC)]
        kr[0] = kr[0] + skip_v[c]
        for n, (j, _, _) in enumerate(_EXTRAS):
            kr[j] = kr[j] + kx_v[c, n, re, :]
            ki[j] = ki[j] + kx_v[c, n, im, :]
        kr, ki = ([kr[0]] + [kr[j] + ki[j - 1] for j in range(1, NC)],
                  [ki[0]] + [ki[j] - kr[j - 1] for j in range(1, NC)])
        half = NC // 2
        for part, k in enumerate((kr, ki)):
            for a in range(half):
                tmp[2 * part, a] = k[2 * a]
                tmp[2 * part, half + a] = (k[2 * a - 1] if a else 0.0) - k[2 * a]
                tmp[2 * part + 1, a] = k[2 * a + 1] - k[2 * a]

        def toeplitz(a, b):
            return [functools.reduce(lambda x, y: x + y, [a[j] * b[i - j] for j in range(i + 1)])
                    for i in range(half)]

        for n in range(3):
            done = 60 + n * PER_PRODUCT
            re, im = rows(done)
            zero = pl.ds(_mult(pace(h0 + done * dh / 100), 8), 8)
            ar, ai = [[tmp[2 * part + n // 2, n % 2 * half + a, zero, :] for a in range(half)] for part in range(2)]
            chunks = lambda e: [[u_v[c, 2 * b + e, r, :] for b in range(half)] for r in (re, im)]
            if n == 0:
                ur, ui = [[x + y for x, y in zip(p, q)] for p, q in zip(chunks(0), chunks(1))]
            else:
                ur, ui = chunks(2 - n)
            k1 = toeplitz(ar, [x + y for x, y in zip(ur, ui)])
            k3 = toeplitz([x + y for x, y in zip(ar, ai)], ui)
            k2 = toeplitz([y - x for x, y in zip(ar, ai)], ur)
            for i in range(half):
                for part, val in enumerate((k1[i] - k3[i], k1[i] + k2[i])):
                    if n == 0:
                        tmp[2 * part + 1, half + i] = val
                    else:
                        put(part, 2 * i + n - 1, tmp[2 * part + 1, half + i] + val)

    def conv_pair(c, s, n, pace, h0, dh):
        def hold(part, i, val):
            hold_v[2 * n + part, i] = val

        def store(part, i, val):
            rows = pl.ds(_mult(part * (T // 2) + s * 8, 8), 8)
            z_v[i, rows, c * 128:(c + 1) * 128] = _pack(hold_v[2 * n + part, i], val)

        conv(c, 2 * s, tmp0_v, pace, h0, dh, hold)
        conv(c, 2 * s + 1, tmp1_v, pace, h0 + 8.1 * dh, dh, store)

    def finish_chunk(i, slot):
        a = jnp.concatenate([jnp.dot(_halves(o_v[slot, e * MO // 2:(e + 1) * MO // 2, :]), _halves(wop_v[...]),
                                     preferred_element_type=F32) for e in range(AB // MO)], axis=0)
        for n in range(AB // T):
            rows = pl.ds(_mult(i * AB + n * T, T), T)
            y = jnp.dot(_halves(gi_v[...]), _halves(z_v[i * (AB // T) + n]), preferred_element_type=F32)
            g = g_v[rows, :]
            for c in range(CT):
                cols = slice(c * 128, (c + 1) * 128)
                mixed = y[:, cols] + g * (a[n * T:(n + 1) * T, cols] - y[:, cols])
                out_v[rows, cols] = mixed.astype(out_v.dtype)

    def out_copy(i):
        rows = pl.ds(_mult(i * AB, AB), AB)
        return pltpu.make_async_copy(out_v.at[rows], out_hbm.at[rows], osems.at[i])

    def loop(n, body):
        jax.lax.fori_loop(0, n, lambda it, _: body(it), None)

    for p, ref in enumerate((ldt_ref, dsk_ref, gw_ref)):
        vec = ref[...].astype(F32).reshape(1, D)
        for c in range(CT):
            row_v[p, c] = jnp.broadcast_to(vec[:, c * 128:(c + 1) * 128], (8, 128))
    zero_s[0] = 0
    for cp in cp_first:
        cp.wait()
    for cp in cp_par:
        cp.start()

    def discretise_step(c):
        @pl.when(c == 1)
        def _():
            for cp in cp_par:
                cp.wait()
            for cp in cp_x:
                cp.start()

        discretise(c)

    loop(CT, discretise_step)
    for n in range(CT, 3 * CT):
        qkv_v[n, 0:HALO, :] = jnp.zeros((HALO, 128), F32)
    P = functools.partial

    def tables(b, slot, pace, h0):
        for k in range(4):
            power_tables(slot, k, b * 32, pace, h0 + H1 * k)

    def taps(b, slot):
        for n in range(2):
            taps16(slot, n, b * 32 + n * 16)

    def input_units(b):
        for u in (2 * b, 2 * b + 1):
            s, c = u // CT, u % CT
            for e in range(RB // T):
                udft(c, s * (RB // T) + e)
            gate(_mult(s * RB + (min if isinstance(c, int) else jnp.minimum)(c, 3) * (RB // 4), RB // 4), RB // 4)

    def phase1(it, more=True):
        pace = _Pacer(zero_s)
        taps(2 * it, 0)
        tables(2 * it + 1, 1, pace, 0)
        input_units(2 * it)
        taps(2 * it + 1, 1)
        if more:
            tables(2 * it + 2, 0, pace, 4 * H1)
        input_units(2 * it + 1)

    n1 = D // 32
    tables(0, 0, lambda h: 0, 0)
    for cp in cp_x:
        cp.wait()
    for cp in cp_rest:
        cp.start()
    loop(n1 // 2 - 1, phase1)
    phase1(n1 // 2 - 1, more=False)

    for cp in cp_rest:
        cp.wait()
    _interleave([P(kdft, 0, j) for j in range(NC)]
                + [P(kdft_extra, c, n) for c in range(CT) for n in range(len(_EXTRAS))],
                [P(permute_w, 1, kt) for kt in range(CT)])

    def keys(c):
        proj_tile(1, c, 0, S)
        permute_w(0, c)
        permute_w(2, c)
        permute_wo(c)

    loop(CT, keys)

    def qv_unit(u):
        s, r = u // (2 * CT), u % (2 * CT)
        for e in range(RB // MR):
            proj_tile(2 * (r // CT), r % CT, _mult(s * RB + e * MR, MR), MR)

    pairs = T // 16
    for c in range(CT):
        def phase2(it, c=c):
            pace = _Pacer(zero_s)
            for n in range(CP):
                s = it * CP + n
                if c + 1 < CT:
                    for e in range(2):
                        qv_unit(2 * (c * pairs + s) + e)
                        kdft(c + 1, 2 * s + e)
                else:
                    qv_unit(2 * c * pairs + s)
            dh = H2 if c + 1 < CT else H2_LAST
            for n in range(CP):
                conv_pair(c, it * CP + n, n, pace, n * 16.2 * dh, dh)

        loop(pairs // CP, phase2)

    def attn_chunk(i, slot, pace, gap):
        for n in range(AB // AR):
            attn_rows(_mult(i * AB + n * AR, AR), AR, isinstance(i, int) and i * AB + n * AR < HALO,
                      pace, n * gap, o_v.at[slot, n * AR // 2:(n + 1) * AR // 2])

    def phase3(i):
        pace = _Pacer(zero_s, loads=False)
        finish_chunk(i - 1, (i - 1) % 2)
        attn_chunk(i, i % 2, pace, H3)
        out_copy(i - 1).start()

    last = S // AB - 1
    for u in range((2 * CT - 1) * pairs, 2 * CT * pairs):
        qv_unit(u)
    attn_chunk(0, 0, _Pacer(zero_s), H3_FIRST)
    loop(last, lambda it: phase3(it + 1))
    finish_chunk(last, last % 2)
    out_copy(last).start()
    for i in range(last + 1):
        out_copy(i).wait()


@jax.jit
def pallas_gated_mix__sliding_local_dilated__ssm_conv_s4__prompt_kernel(
    A_x: jax.Array,
    A_wqkv: jax.Array,
    A_wo: jax.Array,
    B_u: jax.Array,
    B_A_re: jax.Array,
    B_A_im: jax.Array,
    B_B_re: jax.Array,
    B_B_im: jax.Array,
    B_C_re: jax.Array,
    B_C_im: jax.Array,
    B_log_dt: jax.Array,
    B_Dskip: jax.Array,
    gate_w: jax.Array,
):
    del B_u
    assert A_x.shape == (1, S, D) and B_A_re.shape == (D, N) and B_A_re.dtype == BF16
    hbm = pl.BlockSpec(memory_space=pl.ANY)
    vmem = pl.BlockSpec(memory_space=pltpu.VMEM)
    scratch = [
        pltpu.VMEM((S, D), BF16),
        pltpu.VMEM((3, D, D), BF16),
        pltpu.VMEM((D, D), BF16),
        pltpu.VMEM((6, N, D), BF16),
        pltpu.VMEM(_FMATS.shape, jnp.int32),
        pltpu.VMEM(_GINV.shape, jnp.int32),
        pltpu.VMEM((3, CT, 8, 128), F32),
        pltpu.VMEM((8, D, 128), F32),
        pltpu.VMEM((CT, 8, 128), F32),
        pltpu.VMEM((3, D, 128), F32),
        pltpu.VMEM((D, D), jnp.int32),
        pltpu.VMEM((D // 2, D), jnp.int32),
        pltpu.VMEM((D // 2, D), jnp.int32),
        pltpu.VMEM((3 * CT, S + HALO, 128), F32),
        pltpu.VMEM((8, 40, 3 * 128), jnp.int32),
        pltpu.VMEM((8, 40, 3 * 128), jnp.int32),
        pltpu.VMEM((8, 64, 3 * 128), jnp.int32),
        pltpu.VMEM((8, 64, 3 * 128), jnp.int32),
        *[pltpu.VMEM((2, 12, 8, 128), F32)] * 4,
        pltpu.VMEM((4, NC, 8, 128), F32),
        pltpu.VMEM((4, NC, 8, 128), F32),
        pltpu.VMEM((2 * CP, NC, 8, 128), F32),
        pltpu.SMEM((1,), jnp.int32),
        pltpu.VMEM((2, AB // 2, D), jnp.int32),
        pltpu.VMEM((S, 128), F32),
        pltpu.VMEM((5, D // 2, 128), jnp.int32),
        pltpu.VMEM((CT, NC, 2 * T, 128), F32),
        pltpu.VMEM((NC, 2 * T, 128), F32),
        pltpu.VMEM((NC, 2 * T, 128), F32),
        pltpu.VMEM((CT, len(_EXTRAS), 2 * T, 128), F32),
        pltpu.VMEM((NC, T, D), jnp.int32),
        pltpu.VMEM((S, D), BF16),
        pltpu.SemaphoreType.DMA((20,)),
        pltpu.SemaphoreType.DMA((NC,)),
    ]
    out = pl.pallas_call(
        _kernel,
        out_shape=jax.ShapeDtypeStruct((S, D), A_x.dtype),
        in_specs=[hbm] * 9 + [vmem] * 3 + [hbm] * 2,
        out_specs=hbm,
        scratch_shapes=scratch,
        compiler_params=pltpu.CompilerParams(vmem_limit_bytes=100 * 1024 * 1024),
    )(A_x.reshape(S, D), A_wqkv, A_wo, B_A_re.T, B_A_im.T, B_B_re.T, B_B_im.T, B_C_re.T, B_C_im.T,
      B_log_dt, B_Dskip, gate_w, _FMATS, _GINV)
    return out.reshape(1, S, D)
```
